```python
import jax
import jax.numpy as jnp

def _softmax(x, axis=-1):
    return jax.nn.softmax(x, axis=axis)

def _gelu(x):
    return jax.nn.gelu(x, approximate=True)

def _silu(x):
    return jax.nn.silu(x)

def _sigmoid(x):
    return jax.nn.sigmoid(x)

def _layernorm(x, axis=-1, eps=1e-05):
    m = jnp.mean(x, axis=axis, keepdims=True)
    v = jnp.var(x, axis=axis, keepdims=True)
    return (x - m) / jnp.sqrt(v + eps)

def _scatter_add(tgt, idx, src, axis=0):
    return tgt.at[idx].add(src)

def _segment_sum(src, seg, n):
    return jax.ops.segment_sum(src, seg, n)

class _Rng:

    def __init__(self, key):
        self._k = key

    def _next(self):
        self._k, sub = jax.random.split(self._k)
        return sub

    def normal(self, shape):
        return jax.random.normal(self._next(), shape, dtype=jnp.bfloat16)

    def randint(self, lo, hi, shape):
        return jax.random.randint(self._next(), shape, lo, hi, dtype=jnp.int32)

    def uniform(self, shape, lo=0.0, hi=1.0):
        return jax.random.uniform(self._next(), shape, jnp.bfloat16, lo, hi)

    def permutation(self, n):
        return jax.random.permutation(self._next(), n)
kernel_name = 'adaLN_cond__mha_block_cached__moe_arch_mod__decode'

def setup_inputs():
    _rng = _Rng(jax.random.key(int.from_bytes(__import__("os").urandom(4), "little")))
    _w = lambda a: (lambda t: t.astype(jnp.bfloat16) if jnp.issubdtype(t.dtype, jnp.floating) else t)(jnp.asarray(a))

    def _A_setup():
        B, Sq, D = (4, 1, 448)
        H, Sk, Dh = (16, 16384, 256)
        return {'x': _w((lambda *s: _rng.normal(s) * 0.05)(B, Sq, D)), 'k_cache': _w((lambda *s: _rng.normal(s) * 0.05)(B, H, Sk, Dh)), 'v_cache': _w((lambda *s: _rng.normal(s) * 0.05)(B, H, Sk, Dh)), 'wq': _w((lambda *s: _rng.normal(s) * 0.05)(D, H * Dh) * D ** (-0.5)), 'wo': _w((lambda *s: _rng.normal(s) * 0.05)(H * Dh, D) * (H * Dh) ** (-0.5))}
    _A_in = _A_setup()

    def _B_setup():
        B, S, D, F, C = (4, 1, 448, 1792, 1)
        return {'x': _w((lambda *s: _rng.normal(s) * 0.05)(B, S, D)), 'w_r': _w((lambda *s: _rng.normal(s) * 0.05)(D)), 'w_gate': _w((lambda *s: _rng.normal(s) * 0.05)(D, F)), 'w_up': _w((lambda *s: _rng.normal(s) * 0.05)(D, F)), 'w_down': _w((lambda *s: _rng.normal(s) * 0.05)(F, D))}
    _B_in = _B_setup()
    return {'A_x': _A_in['x'], 'A_k_cache': _A_in['k_cache'], 'A_v_cache': _A_in['v_cache'], 'A_wq': _A_in['wq'], 'A_wo': _A_in['wo'], 'B_x': _B_in['x'], 'B_w_r': _B_in['w_r'], 'B_w_gate': _B_in['w_gate'], 'B_w_up': _B_in['w_up'], 'B_w_down': _B_in['w_down'], 'c': _w((lambda *s: _rng.normal(s) * 0.05)(4, 448)), 'w_mod': _w((lambda *s: _rng.normal(s) * 0.05)(448, 6 * 448) * 448 ** (-0.5))}

def reference(A_x, A_k_cache, A_v_cache, A_wq, A_wo, B_x, B_w_r, B_w_gate, B_w_up, B_w_down, c, w_mod):

    def _A_ref(x, k_cache, v_cache, wq, wo):
        B, Sq, D = x.shape
        H, Dh = (16, 256)
        q = (lambda x, *d: x.transpose(*d))((x @ wq).reshape(B, Sq, H, Dh), 0, 2, 1, 3)
        scores = jnp.einsum('bhqd,bhkd->bhqk', q, k_cache) * Dh ** (-0.5)
        p = _softmax(scores, axis=-1)
        o = jnp.einsum('bhqk,bhkd->bhqd', p, v_cache)
        return (lambda x, *d: x.transpose(*d))(o, 0, 2, 1, 3).reshape(B, Sq, H * Dh) @ wo

    def _B_ref(x, w_r, w_gate, w_up, w_down):
        B, S, D = x.shape
        C = 1
        r = x @ w_r
        idx = jnp.argsort(-r, axis=-1)[:, :C]
        idx_e = jnp.repeat(idx.reshape(B, C, 1), D, axis=2)
        x_sel = jnp.take_along_axis(x, idx_e, axis=1)
        g = _silu(x_sel @ w_gate)
        u = x_sel @ w_up
        y = g * u @ w_down
        r_sel = _sigmoid(jnp.take_along_axis(r, idx, axis=1))
        y = y * r_sel.reshape(B, C, 1)
        b_off = (jnp.arange(B) * S).reshape(B, 1)
        flat_idx = (idx + b_off).reshape(B * C)
        zero = (x * 0.0).reshape(B * S, D)
        upd = _scatter_add(zero, flat_idx, y.reshape(B * C, D), axis=0)
        return x + upd.reshape(B, S, D)
    x = A_x
    mod = (_silu(c) @ w_mod).reshape(c.shape[0], 6, 1, -1)
    sa, ca, ga, sb, cb, gb = (mod[:, 0].copy(), mod[:, 1].copy(), mod[:, 2].copy(), mod[:, 3].copy(), mod[:, 4].copy(), mod[:, 5].copy())
    h = _layernorm(x, axis=-1) * (1 + ca) + sa
    x = x + ga * _A_ref(h, A_k_cache, A_v_cache, A_wq, A_wo)
    h = _layernorm(x, axis=-1) * (1 + cb) + sb
    x = x + gb * _B_ref(h, B_w_r, B_w_gate, B_w_up, B_w_down)
    return x
```

```python
import functools
import jax
import jax.numpy as jnp
import numpy as np
from jax import lax
import jax.experimental.pallas as pl
import jax.experimental.pallas.tpu as pltpu

B, D, H, SK, DH, F = 4, 448, 16, 16384, 256, 1792
R = 8


def make(T=2048, NBUF=4, P=64, pat="1110", unroll=1):
    NC = SK // T
    TOTAL = B * H * 2 * NC
    f32, bf16 = jnp.float32, jnp.bfloat16

    def rnd(x):
        return x.astype(bf16).astype(f32)

    def layernorm(x):
        m = jnp.mean(x, axis=-1, keepdims=True)
        xc = x - m
        v = jnp.mean(xc * xc, axis=-1, keepdims=True)
        return xc / jnp.sqrt(v + 1e-5)

    def kernel(x_ref, c_ref, wr_ref, k_hbm, v_hbm, wq_hbm, wo_hbm, wg_hbm, wu_hbm, wd_hbm, wm_hbm,
               o_ref,
               buf, sems, wq_s, wo_s, wg_s, wu_s, wd_s, wm_s, wsems,
               q_s, s_s, oh_s, mod_s, att_s):
        def start(i):
            slot = i % NBUF
            hb = i // (2 * NC)
            r = i % (2 * NC)
            isv = r // NC
            h = hb // B
            b = hb % B
            row = (b * H + h) * SK + (r % NC) * T

            def go(src):
                for j in range(T // P):
                    pltpu.make_async_copy(
                        src.at[pl.ds(pl.multiple_of(row + j * P, P), P), :],
                        buf.at[slot, pl.ds(j * P, P), :],
                        sems.at[slot]).start(priority=int(pat[j % len(pat)]))
            if isinstance(i, int):
                go(v_hbm if isv else k_hbm)
            else:
                @pl.when(isv == 0)
                def _():
                    go(k_hbm)

                @pl.when(isv == 1)
                def _():
                    go(v_hbm)

        def wait(i):
            slot = i % NBUF
            pltpu.make_async_copy(buf.at[slot], buf.at[slot], sems.at[slot]).wait()

        def next_start(i):
            @pl.when(i + NBUF - 1 < TOTAL)
            def _():
                start(i + NBUF - 1)

        cp_m = pltpu.make_async_copy(wm_hbm, wm_s, wsems.at[0])
        cp_q = pltpu.make_async_copy(wq_hbm, wq_s, wsems.at[1])
        cp_o = pltpu.make_async_copy(wo_hbm, wo_s, wsems.at[2])
        cp_g = pltpu.make_async_copy(wg_hbm, wg_s, wsems.at[3])
        cp_u = pltpu.make_async_copy(wu_hbm, wu_s, wsems.at[4])
        cp_d = pltpu.make_async_copy(wd_hbm, wd_s, wsems.at[5])
        cp_m.start()
        cp_q.start()
        for i in range(NBUF - 1):
            start(i)
        cp_o.start()
        cp_g.start()
        cp_u.start()
        cp_d.start()

        zpad = jnp.zeros((R - B, D), f32)
        x = jnp.concatenate([x_ref[...].astype(f32), zpad], axis=0)
        c = jnp.concatenate([c_ref[...].astype(f32), zpad], axis=0)
        sc = c * jax.nn.sigmoid(c)
        cp_m.wait()
        mod = jnp.dot(sc.astype(bf16), wm_s[...], preferred_element_type=f32)
        for j in range(6):
            mod_s[j] = mod[:, j * D:(j + 1) * D]
        hA = layernorm(x) * (1.0 + mod_s[1]) + mod_s[0]
        cp_q.wait()
        q = jnp.dot(hA.astype(bf16), wq_s[...], preferred_element_type=f32)
        for h in range(H):
            q_s[h] = q[:, h * DH:(h + 1) * DH].astype(bf16)
        att_s[...] = jnp.zeros((R, D), f32)
        cp_o.wait()

        rows = lax.broadcasted_iota(jnp.int32, (R, DH), 0)

        def head_body(h, _):
            oh_s[...] = jnp.zeros((R, DH), f32)

            def batch_body(b, _):
                g0 = (h * B + b) * (2 * NC)
                qh = q_s[h]

                def k_body(ci, m):
                    g = g0 + ci
                    next_start(g)
                    wait(g)
                    kc = buf[g % NBUF]
                    s = lax.dot_general(qh, kc, (((1,), (1,)), ((), ())), preferred_element_type=f32)
                    s_s[ci] = s
                    for j in range(T // 128):
                        m = jnp.maximum(m, s[:, j * 128:(j + 1) * 128])
                    return m
                m = lax.fori_loop(0, NC, k_body, jnp.full((R, 128), -jnp.inf, f32), unroll=unroll)
                m = jnp.max(m, axis=-1, keepdims=True) * (DH ** -0.5)

                def v_body(ci, carry):
                    l, acc = carry
                    g = g0 + NC + ci
                    next_start(g)
                    p = jnp.exp(s_s[ci] * (DH ** -0.5) - m)
                    for j in range(T // 128):
                        l = l + p[:, j * 128:(j + 1) * 128]
                    wait(g)
                    vc = buf[g % NBUF]
                    acc = acc + jnp.dot(p.astype(bf16), vc, preferred_element_type=f32)
                    return l, acc
                l, acc = lax.fori_loop(0, NC, v_body, (jnp.zeros((R, 128), f32), jnp.zeros((R, DH), f32)), unroll=unroll)
                l = jnp.sum(l, axis=-1, keepdims=True)
                oh_s[...] = jnp.where(rows == b, acc / l, oh_s[...])
                return 0
            lax.fori_loop(0, B, batch_body, 0)
            att_s[...] += lax.dot_general(oh_s[...].astype(bf16), wo_s[:, pl.ds(pl.multiple_of(h * DH, DH), DH)],
                                          (((1,), (1,)), ((), ())), preferred_element_type=f32)
            return 0
        lax.fori_loop(0, H, head_body, 0)

        x = jnp.concatenate([x_ref[...].astype(f32), zpad], axis=0)
        x = x + mod_s[2] * att_s[...]
        hB = layernorm(x) * (1.0 + mod_s[4]) + mod_s[3]
        r = jnp.sum(hB * wr_ref[...].astype(f32), axis=-1, keepdims=True)
        hb16 = hB.astype(bf16)
        cp_g.wait()
        cp_u.wait()
        cp_d.wait()
        g = jnp.dot(hb16, wg_s[...], preferred_element_type=f32)
        u = jnp.dot(hb16, wu_s[...], preferred_element_type=f32)
        gu = (g * jax.nn.sigmoid(g)) * u
        y = lax.dot_general(gu.astype(bf16), wd_s[...], (((1,), (1,)), ((), ())), preferred_element_type=f32)
        y = y * jax.nn.sigmoid(r)
        out = x + mod_s[5] * (hB + y)
        o_ref[...] = out[:B].astype(o_ref.dtype)

    anyspec = pl.BlockSpec(memory_space=pltpu.HBM)
    vm = pl.BlockSpec(memory_space=pltpu.VMEM)
    call = pl.pallas_call(
        kernel,
        in_specs=[vm, vm, vm] + [anyspec] * 8,
        out_specs=vm,
        out_shape=jax.ShapeDtypeStruct((B, D), bf16),
        scratch_shapes=[
            pltpu.VMEM((NBUF, T, DH), bf16), pltpu.SemaphoreType.DMA((NBUF,)),
            pltpu.VMEM((D, H * DH), bf16), pltpu.VMEM((D, H * DH), bf16),
            pltpu.VMEM((D, F), bf16), pltpu.VMEM((D, F), bf16), pltpu.VMEM((D, F), bf16),
            pltpu.VMEM((D, 6 * D), bf16), pltpu.SemaphoreType.DMA((6,)),
            pltpu.VMEM((H, R, DH), bf16), pltpu.VMEM((NC, R, T), f32), pltpu.VMEM((R, DH), f32),
            pltpu.VMEM((6, R, D), f32), pltpu.VMEM((R, D), f32),
        ],
        compiler_params=pltpu.CompilerParams(vmem_limit_bytes=100 * 1024 * 1024),
    )

    @jax.jit
    def f(A_x, A_k_cache, A_v_cache, A_wq, A_wo, B_x, B_w_r, B_w_gate, B_w_up, B_w_down, c, w_mod):
        out = call(A_x.reshape(B, D), c, B_w_r.reshape(1, D),
                   A_k_cache.reshape(B * H * SK, DH), A_v_cache.reshape(B * H * SK, DH),
                   A_wq, A_wo.T, B_w_gate, B_w_up, B_w_down.T, w_mod)
        return out.reshape(B, 1, D)
    return f


pallas_adaLN_cond__mha_block_cached__moe_arch_mod__decode_kernel = make()
```

```python
import jax
import jax.numpy as jnp
from jax import lax
import jax.experimental.pallas as pl
import jax.experimental.pallas.tpu as pltpu

B, D, H, SK, DH, F = 4, 448, 16, 16384, 256, 1792
R = 8


def make(T=4096, pat="1120_1121", unroll=1, nobc=0):
    NC = SK // T
    f32, bf16 = jnp.float32, jnp.bfloat16
    NT = (((1,), (1,)), ((), ()))

    def layernorm(x):
        m = jnp.mean(x, axis=-1, keepdims=True)
        xc = x - m
        v = jnp.mean(xc * xc, axis=-1, keepdims=True)
        return xc / jnp.sqrt(v + 1e-5)

    def kernel(x_ref, c_ref, wr_ref, k_hbm, v_hbm, wq_hbm, wo_hbm, wg_hbm, wu_hbm, wd_hbm, wm_hbm,
               o_ref,
               kbuf, vbuf, ksems, vsems, wq_s, wo_s, wg_s, wu_s, wd_s, wm_s, wsems,
               q_s, s_s, oh_s, mod_s, att_s):
        def start(src, dst, sems, row0, ci):
            items = [(int(x[:-1]), int(x[-1])) for x in pat.split("_")]
            off = 0
            j = 0
            while off < T:
                n, pr = items[j % len(items)]
                n = min(n, T - off)
                pltpu.make_async_copy(
                    src.at[pl.ds(pl.multiple_of(row0 + ci * T + off, 8), n), :],
                    dst.at[ci, pl.ds(off, n), :],
                    sems.at[ci]).start(priority=pr)
                off += n
                j += 1

        def wait(dst, sems, ci):
            pltpu.make_async_copy(dst.at[ci], dst.at[ci], sems.at[ci]).wait()

        cp_m = pltpu.make_async_copy(wm_hbm, wm_s, wsems.at[0])
        cp_q = pltpu.make_async_copy(wq_hbm, wq_s, wsems.at[1])
        cp_o = pltpu.make_async_copy(wo_hbm, wo_s, wsems.at[2])
        cp_g = pltpu.make_async_copy(wg_hbm, wg_s, wsems.at[3])
        cp_u = pltpu.make_async_copy(wu_hbm, wu_s, wsems.at[4])
        cp_d = pltpu.make_async_copy(wd_hbm, wd_s, wsems.at[5])
        cp_m.start()
        cp_q.start()
        for ci in range(NC):
            pltpu.make_async_copy(k_hbm.at[pl.ds(ci * T, T), :], kbuf.at[ci], ksems.at[ci]).start(priority=ci % 2)
        cp_o.start()

        zpad = jnp.zeros((R - B, D), f32)
        x = jnp.concatenate([x_ref[...].astype(f32), zpad], axis=0)
        c = jnp.concatenate([c_ref[...].astype(f32), zpad], axis=0)
        sc = c * jax.nn.sigmoid(c)
        cp_m.wait()
        mod = jnp.dot(sc.astype(bf16), wm_s[...], preferred_element_type=f32)
        for j in range(6):
            mod_s[j] = mod[:, j * D:(j + 1) * D]
        hA = layernorm(x) * (1.0 + mod_s[1]) + mod_s[0]
        cp_q.wait()
        q = jnp.dot(hA.astype(bf16), wq_s[...], preferred_element_type=f32)
        for h in range(H):
            q_s[h] = q[:, h * DH:(h + 1) * DH].astype(bf16)
        att_s[...] = jnp.zeros((R, D), f32)
        cp_o.wait()

        rows = lax.broadcasted_iota(jnp.int32, (R, DH), 0)

        def hb_body(hb, _):
            hb1 = hb + 1
            h = hb // B
            b = hb % B
            row0 = (b * H + h) * SK
            row1 = ((hb1 % B) * H + hb1 // B) * SK
            qh = q_s[h]

            def k_body(ci, m):
                start(v_hbm, vbuf, vsems, row0, ci)
                wait(kbuf, ksems, ci)
                s = lax.dot_general(qh, kbuf[ci], NT, preferred_element_type=f32)
                s_s[ci] = s
                for j in range(T // 128):
                    m = jnp.maximum(m, s[:, j * 128:(j + 1) * 128])
                return m
            m = lax.fori_loop(0, NC, k_body, jnp.full((R, 128), -jnp.inf, f32), unroll=unroll)
            m = jnp.max(m, axis=-1, keepdims=True) * (DH ** -0.5)

            def v_body(ci, carry):
                l, acc = carry

                @pl.when(hb1 < H * B)
                def _():
                    start(k_hbm, kbuf, ksems, row1, ci)

                @pl.when(jnp.logical_and(hb1 == H * B, ci == 0))
                def _():
                    cp_g.start(priority=1)
                    cp_u.start()
                    cp_d.start(priority=1)
                p = jnp.exp(s_s[ci] * (DH ** -0.5) - m)
                for j in range(T // 128):
                    l = l + p[:, j * 128:(j + 1) * 128]
                wait(vbuf, vsems, ci)
                acc = acc + jnp.dot(p.astype(bf16), vbuf[ci], preferred_element_type=f32)
                return l, acc
            l, acc = lax.fori_loop(0, NC, v_body, (jnp.zeros((R, 128), f32), jnp.zeros((R, DH), f32)), unroll=unroll)
            l = jnp.sum(l, axis=-1, keepdims=True)

            @pl.when(b == 0)
            def _():
                oh_s[...] = acc / l

            @pl.when(b > 0)
            def _():
                oh_s[...] = jnp.where(rows == b, acc / l, oh_s[...])

            @pl.when(b == B - 1)
            def _():
                att_s[...] += lax.dot_general(oh_s[...].astype(bf16), wo_s[:, pl.ds(pl.multiple_of(h * DH, DH), DH)],
                                              NT, preferred_element_type=f32)
            return 0
        lax.fori_loop(0, H * B, hb_body, 0)

        x = jnp.concatenate([x_ref[...].astype(f32), zpad], axis=0)
        x = x + mod_s[2] * att_s[...]
        hB = layernorm(x) * (1.0 + mod_s[4]) + mod_s[3]
        r = jnp.sum(hB * wr_ref[...].astype(f32).reshape(1, D), axis=-1, keepdims=True)
        hb16 = hB.astype(bf16)
        cp_g.wait()
        cp_u.wait()
        g = jnp.dot(hb16, wg_s[...], preferred_element_type=f32)
        u = jnp.dot(hb16, wu_s[...], preferred_element_type=f32)
        gu = (g * jax.nn.sigmoid(g)) * u
        cp_d.wait()
        y = lax.dot_general(gu.astype(bf16), wd_s[...], NT, preferred_element_type=f32)
        y = y * jax.nn.sigmoid(r)
        out = x + mod_s[5] * (hB + y)
        o_ref[...] = out[:B].astype(o_ref.dtype)

    anyspec = pl.BlockSpec(memory_space=pltpu.HBM)
    vm = pl.BlockSpec(memory_space=pltpu.VMEM)
    call = pl.pallas_call(
        kernel,
        in_specs=[vm, vm, vm] + [anyspec] * 8,
        out_specs=vm,
        out_shape=jax.ShapeDtypeStruct((B, D), bf16),
        scratch_shapes=[
            pltpu.VMEM((NC, T, DH), bf16), pltpu.VMEM((NC, T, DH), bf16),
            pltpu.SemaphoreType.DMA((NC,)), pltpu.SemaphoreType.DMA((NC,)),
            pltpu.VMEM((D, H * DH), bf16), pltpu.VMEM((D, H * DH), bf16),
            pltpu.VMEM((D, F), bf16), pltpu.VMEM((D, F), bf16), pltpu.VMEM((D, F), bf16),
            pltpu.VMEM((D, 6 * D), bf16), pltpu.SemaphoreType.DMA((6,)),
            pltpu.VMEM((H, R, DH), bf16), pltpu.VMEM((NC, R, T), f32), pltpu.VMEM((R, DH), f32),
            pltpu.VMEM((6, R, D), f32), pltpu.VMEM((R, D), f32),
        ],
        compiler_params=pltpu.CompilerParams(vmem_limit_bytes=100 * 1024 * 1024, disable_bounds_checks=bool(nobc)),
    )

    @jax.jit
    def f(A_x, A_k_cache, A_v_cache, A_wq, A_wo, B_x, B_w_r, B_w_gate, B_w_up, B_w_down, c, w_mod):
        out = call(A_x.reshape(B, D), c, B_w_r,
                   A_k_cache.reshape(B * H * SK, DH), A_v_cache.reshape(B * H * SK, DH),
                   A_wq, A_wo.T, B_w_gate, B_w_up, B_w_down.T, w_mod)
        return out.reshape(B, 1, D)
    return f


pallas_adaLN_cond__mha_block_cached__moe_arch_mod__decode_kernel = make()
```
